```python
import os as _os
_os.environ.setdefault("JAX_PLATFORMS", "cpu")
import jax
import jax.numpy as jnp

def _softmax(x, axis=-1):
    return jax.nn.softmax(x, axis=axis)
def _gelu(x):
    return jax.nn.gelu(x, approximate=True)
def _silu(x):
    return jax.nn.silu(x)
def _sigmoid(x):
    return jax.nn.sigmoid(x)
def _layernorm(x, axis=-1, eps=1e-5):
    m = jnp.mean(x, axis=axis, keepdims=True)
    v = jnp.var(x, axis=axis, keepdims=True)
    return (x - m) / jnp.sqrt(v + eps)
def _scatter_add(tgt, idx, src, axis=0):
    return tgt.at[idx].add(src)
def _segment_sum(src, seg, n):
    return jax.ops.segment_sum(src, seg, n)
class _Rng:
    def __init__(self, key):
        self._k = key
    def _next(self):
        self._k, sub = jax.random.split(self._k)
        return sub
    def normal(self, shape):
        return jax.random.normal(self._next(), shape, dtype=jnp.bfloat16)
    def randint(self, lo, hi, shape):
        return jax.random.randint(self._next(), shape, lo, hi, dtype=jnp.int32)
    def uniform(self, shape, lo=0.0, hi=1.0):
        return jax.random.uniform(self._next(), shape, jnp.bfloat16, lo, hi)
    def permutation(self, n):
        return jax.random.permutation(self._next(), n)


kernel_name = 'parallel_sum__sliding_local_dilated__dense_activation_mish__prompt'

def setup_inputs():
    _rng = _Rng(jax.random.key(int.from_bytes(__import__("os").urandom(4), "little")))
    _w = (lambda a: (lambda t: t.astype(jnp.bfloat16) if jnp.issubdtype(t.dtype, jnp.floating) else t)(jnp.asarray(a)))
    def _A_setup():
        B, S, D = 1, 2048, 576
        return {
            "x": _w((lambda *s: _rng.normal(s) * 0.05)(B, S, D)),
            "wqkv": _w((lambda *s: _rng.normal(s) * 0.05)(D, 3 * D)),
            "wo": _w((lambda *s: _rng.normal(s) * 0.05)(D, D)),
        }
    _A_in = _A_setup()

    def _B_setup():
        B, S, D, F = 1, 2048, 576, 4608
        return {
            "x": _w((lambda *s: _rng.normal(s) * 0.05)(B, S, D)),
            "w1": _w((lambda *s: _rng.normal(s) * 1.6)(D, F) * (D ** -0.5)),
            "b1": _w((lambda *s: _rng.normal(s) * 0.2)(F)),
            "w2": _w((lambda *s: _rng.normal(s) * 0.2)(F, D) * (F ** -0.5)),
        }
    _B_in = _B_setup()

    return {
        "A_x": _A_in["x"],
        "A_wqkv": _A_in["wqkv"],
        "A_wo": _A_in["wo"],
        "B_x": _B_in["x"],
        "B_w1": _B_in["w1"],
        "B_b1": _B_in["b1"],
        "B_w2": _B_in["w2"],
    }

def reference(A_x, A_wqkv, A_wo, B_x, B_w1, B_b1, B_w2):
    def _A_ref(x, wqkv, wo):
        B, S, D = x.shape
        H = 32; Dh = D // H
        W, dil = 8, 2
        qkv = (lambda x, *d: x.transpose(*d))((x @ wqkv).reshape(B, S, 3, H, Dh), 2, 0, 3, 1, 4)
        q, k, v = qkv[0], qkv[1], qkv[2]
        scale = Dh ** -0.5
        pos = jnp.arange(S)
        off = jnp.arange(W) * dil
        idx = pos[:, None] - off[None, :]
        mask = idx >= 0
        idx_c = jnp.where(mask, idx, 0).reshape(-1)
        kg = k[:, :, idx_c, :].reshape(B, H, S, W, Dh)
        vg = v[:, :, idx_c, :].reshape(B, H, S, W, Dh)
        logits = jnp.einsum("bhsd,bhswd->bhsw", q, kg) * scale
        logits = jnp.where(mask[None, None, :, :], logits, -1e9)
        attn = _softmax(logits, axis=-1)
        o = jnp.einsum("bhsw,bhswd->bhsd", attn, vg)
        return (lambda x, *d: x.transpose(*d))(o, 0, 2, 1, 3).reshape(B, S, D) @ wo

    def _B_ref(x, w1, b1, w2):
        h = jnp.einsum("bsd,df->bsf", x, w1) + b1
        sp = jnp.log1p(jnp.exp(-jnp.abs(h))) + jnp.where(h > 0, h, jnp.zeros_like(h))
        act = h * jnp.tanh(sp)
        return jnp.einsum("bsf,fd->bsd", act, w2)

    x = A_x
    xn = _layernorm(x, axis=-1)
    return x + _A_ref(xn, A_wqkv, A_wo) + _B_ref(xn, B_w1, B_b1, B_w2)
```

```python
import functools
import jax
import jax.numpy as jnp
from jax import lax
import jax.experimental.pallas as pl
import jax.experimental.pallas.tpu as pltpu

S, D, F = 2048, 576, 4608
H, DH, W, DIL = 32, 18, 8, 2
T = 512
FC = 512
NB = T // 128
KP = 592
EPS = 1e-5
f32 = jnp.float32
bf16 = jnp.bfloat16
TN = (((0,), (0,)), ((), ()))


def mish(h):
    e = jnp.exp(jnp.minimum(h, 30.0))
    n = e * (e + 2.0)
    return h * (n * pl.reciprocal(n + 2.0, approx=True))


def kernel(x_ref, wqkv_ref, wo_ref, w1_ref, b1_ref, w2t_ref, out_ref,
           w1e_ref, wof_ref, wop_ref, xn_ref, q_ref, k_ref, v_ref, o_ref):
    i = pl.program_id(0)

    @pl.when(i == 0)
    def _():
        w1e_ref[0:D, :] = w1_ref[...]
        row = lax.broadcasted_iota(jnp.int32, (16, F), 0)
        w1e_ref[D:KP, :] = jnp.where(row == 0, b1_ref[...].astype(f32), 0.0).astype(bf16)
        rowx = lax.broadcasted_iota(jnp.int32, (16, T), 0)
        xn_ref[D:KP, :] = jnp.where(rowx == 0, 1.0, 0.0).astype(bf16)
        for n in range(5):
            nw = min(128, D - n * 128)
            wof_ref[n, :, 0:nw] = wo_ref[:, n * 128:n * 128 + nw].astype(f32)
        for n in range(5):
            nw = min(128, D - n * 128)
            for d in range(DH):
                wop_ref[d * H:(d + 1) * H, n * 128:n * 128 + nw] = wof_ref[n, pl.ds(d, H, stride=DH), :][:, 0:nw].astype(bf16)
        k_ref[0] = jnp.zeros((D, 128), f32)
        v_ref[0] = jnp.zeros((D, 128), f32)

    @pl.when(i > 0)
    def _():
        k_ref[0] = k_ref[NB]
        v_ref[0] = v_ref[NB]

    x = x_ref[...].astype(f32)
    mean = jnp.mean(x, axis=0, keepdims=True)
    xc = x - mean
    var = jnp.mean(xc * xc, axis=0, keepdims=True)
    xn = (xc * lax.rsqrt(var + EPS)).astype(bf16)
    xn_ref[0:D, :] = xn

    qkv = lax.dot_general(wqkv_ref[...], xn, TN, preferred_element_type=f32)
    for j in range(NB):
        q_ref[j] = qkv[0:D, j * 128:(j + 1) * 128]
        k_ref[j + 1] = qkv[D:2 * D, j * 128:(j + 1) * 128]
        v_ref[j + 1] = qkv[2 * D:3 * D, j * 128:(j + 1) * 128]

    cexp = (DH ** -0.5) * 1.4426950408889634
    neg = -1e9 * (DH ** 0.5)
    G = 16
    lane = lax.broadcasted_iota(jnp.int32, (G, 128), 1)

    def shifted(prev, cur, w):
        if w == 0:
            return cur
        m = jnp.where(lane >= 128 - DIL * w, prev, cur)
        return pltpu.roll(m, DIL * w, 1)

    for j in range(T // 128):
        for g in range(H // G):
            L = [None] * W
            for d in range(DH):
                rows = pl.ds(d + g * G * DH, G, stride=DH)
                q = q_ref[j, rows, :]
                prev = k_ref[j, rows, :]
                cur = k_ref[j + 1, rows, :]
                for w in range(W):
                    t = q * shifted(prev, cur, w)
                    L[w] = t if L[w] is None else L[w] + t
            if j == 0:
                pos = i * T + lane
                for w in range(1, W):
                    L[w] = jnp.where(pos >= DIL * w, L[w], neg)
            m = L[0]
            for w in range(1, W):
                m = jnp.maximum(m, L[w])
            P = [jnp.exp2((l - m) * cexp) for l in L]
            den = P[0]
            for w in range(1, W):
                den = den + P[w]
            inv = 1.0 / den
            P = [p * inv for p in P]
            for d in range(DH):
                rows = pl.ds(d + g * G * DH, G, stride=DH)
                prev = v_ref[j, rows, :]
                cur = v_ref[j + 1, rows, :]
                acc = None
                for w in range(W):
                    t = P[w] * shifted(prev, cur, w)
                    acc = t if acc is None else acc + t
                o_ref[d * H + g * G: d * H + (g + 1) * G, j * 128:(j + 1) * 128] = acc.astype(bf16)

    acc = x
    for c in range(F // FC):
        h = lax.dot_general(w1e_ref[:, c * FC:(c + 1) * FC], xn_ref[...], TN, preferred_element_type=f32)
        a = mish(h).astype(bf16)
        acc = acc + jnp.dot(w2t_ref[:, c * FC:(c + 1) * FC], a, preferred_element_type=f32)
    acc = acc + lax.dot_general(wop_ref[...], o_ref[...], TN, preferred_element_type=f32)
    out_ref[...] = acc.astype(bf16)


@jax.jit
def pallas_parallel_sum__sliding_local_dilated__dense_activation_mish__prompt_kernel(
    A_x, A_wqkv, A_wo, B_x, B_w1, B_b1, B_w2):
    b1 = B_b1.reshape(1, F)
    xt = jnp.swapaxes(A_x, 1, 2)
    w2t = B_w2.T
    const = lambda i: (0, 0)
    one = pl.Buffered(1)
    outt = pl.pallas_call(
        kernel,
        grid=(S // T,),
        in_specs=[
            pl.BlockSpec((None, D, T), lambda i: (0, 0, i)),
            pl.BlockSpec((D, 3 * D), const, pipeline_mode=one),
            pl.BlockSpec((D, D), const, pipeline_mode=one),
            pl.BlockSpec((D, F), const, pipeline_mode=one),
            pl.BlockSpec((1, F), const, pipeline_mode=one),
            pl.BlockSpec((D, F), const, pipeline_mode=one),
        ],
        out_specs=pl.BlockSpec((None, D, T), lambda i: (0, 0, i)),
        out_shape=jax.ShapeDtypeStruct((1, D, S), bf16),
        scratch_shapes=[
            pltpu.VMEM((KP, F), bf16),
            pltpu.VMEM((5, D, 128), f32),
            pltpu.VMEM((D, D), bf16),
            pltpu.VMEM((KP, T), bf16),
            pltpu.VMEM((NB, D, 128), f32),
            pltpu.VMEM((NB + 1, D, 128), f32),
            pltpu.VMEM((NB + 1, D, 128), f32),
            pltpu.VMEM((D, T), bf16),
        ],
        compiler_params=pltpu.CompilerParams(
            dimension_semantics=("arbitrary",),
            vmem_limit_bytes=100 * 1024 * 1024,
        ),
    )(xt, A_wqkv, A_wo, B_w1, b1, w2t)
    return jnp.swapaxes(outt, 1, 2)
```

```python
import jax
import jax.numpy as jnp
from jax import lax
import jax.experimental.pallas as pl
import jax.experimental.pallas.tpu as pltpu

S, D, F = 2048, 576, 4608
H, DH, W, DIL = 32, 18, 8, 2
T = 256
NT = S // T
NB = T // 128
KP = 640
G = 8
F_CHUNKS = (2560, 1024, 1024)
QP = ((0, 384), (384, 1024), (1024, 1728))
EPS = 1e-5
LOG2E = 1.4426950408889634
LOG2E_HI = 1.4453125
LOG2E_LO = LOG2E - LOG2E_HI

f32 = jnp.float32
bf16 = jnp.bfloat16
u32 = jnp.uint32


def _pk(x):
    return pltpu.bitcast(x, u32)


def _unpk(x):
    return pltpu.bitcast(x, bf16)


def _mish2(g):
    e = jnp.exp2(jnp.minimum(g, 40.0))
    n = e * (e + 2.0)
    return g * (n * pl.reciprocal(n + 2.0, approx=True))


def _kernel(x_hbm, wqkv_hbm, wo_hbm, w1_hbm, b1_hbm, w2t_hbm, out_ref,
            x_ref, wqkv_ref, wo_ref, w1_ref, b1_ref, w2t_ref,
            w1t_ref, wqkvt_ref, wof_ref, wopt_ref, xg_ref, q_ref, k_ref, v_ref, o_ref, sems):
    step = pl.program_id(0)

    def x_copy(tt):
        return pltpu.make_async_copy(x_hbm.at[0, :, pl.ds(tt * T, T)], x_ref.at[tt], sems.at[tt])

    def wqkv_copy(p):
        a, b = QP[p]
        return pltpu.make_async_copy(
            wqkv_hbm.at[:, pl.ds(a, b - a)], wqkv_ref.at[:, pl.ds(a, b - a)], sems.at[NT + p])

    def layernorm(tt, fast=False):
        if fast:
            def colsum(parts):
                while len(parts) > 1:
                    parts = [parts[k] + parts[k + 1] for k in range(0, len(parts) - 1, 2)] + (
                        [parts[-1]] if len(parts) % 2 else [])
                return jnp.sum(parts[0], axis=0, keepdims=True)

            n1, n2, n3 = D // 4, D // 6, D // 3
            mean = colsum([jnp.sum(x_ref[tt, a:a + n1, :].astype(f32).reshape(n1 // 8, 8, T), axis=0)
                           for a in range(0, D, n1)]) * (1.0 / D)
            parts = []
            for a in range(0, D, n2):
                xc = x_ref[tt, a:a + n2, :].astype(f32) - mean
                parts.append(jnp.sum((xc * xc).reshape(n2 // 8, 8, T), axis=0))
            rstd = lax.rsqrt(colsum(parts) * (1.0 / D) + EPS) * LOG2E
            for a in range(0, D, n3):
                xc = x_ref[tt, a:a + n3, :].astype(f32) - mean
                xg_ref[tt, a // 2:(a + n3) // 2, :] = _pk((xc * rstd).astype(bf16))
        else:
            x = x_ref[tt].astype(f32)
            mean = jnp.sum(x, axis=0, keepdims=True) * (1.0 / D)
            xc = x - mean
            rstd = lax.rsqrt(jnp.sum(xc * xc, axis=0, keepdims=True) * (1.0 / D) + EPS) * LOG2E
            xg_ref[tt, 0:D // 2, :] = _pk((xc * rstd).astype(bf16))
        row = lax.broadcasted_iota(jnp.int32, (KP - D, T), 0)
        xg_ref[tt, D // 2:KP // 2, :] = _pk(
            jnp.where(row == 0, LOG2E_HI, jnp.where(row == 1, LOG2E_LO, 0.0)).astype(bf16))

    def qkv(tiles, a, b):
        xg = _unpk(jnp.concatenate([xg_ref[tt, 0:D // 2, :] for tt in tiles], axis=1))
        val = jnp.dot(_unpk(wqkvt_ref[a // 2:b // 2, :]), xg, preferred_element_type=f32)
        for sec, ref, off in ((0, q_ref, 0), (1, k_ref, 1), (2, v_ref, 1)):
            lo, hi = max(a, sec * D), min(b, (sec + 1) * D)
            if lo >= hi:
                continue
            for j in range(len(tiles) * NB):
                ref[tiles[0] * NB + j + off, lo - sec * D:hi - sec * D, :] = (
                    val[lo - a:hi - a, j * 128:(j + 1) * 128])

    @pl.when(step == 0)
    def _phase_a():
        wo_copy = pltpu.make_async_copy(wo_hbm, wo_ref, sems.at[NT + 3])
        b1_copy = pltpu.make_async_copy(b1_hbm, b1_ref, sems.at[NT + 4])
        w1_copy = pltpu.make_async_copy(w1_hbm, w1_ref, sems.at[NT + 5])
        w2_copy = pltpu.make_async_copy(w2t_hbm, w2t_ref, sems.at[NT + 6])

        x_copy(0).start()
        x_copy(1).start()
        for p in range(3):
            wqkv_copy(p).start()
        for tt in range(2, NT):
            x_copy(tt).start()
        wo_copy.start()
        b1_copy.start()
        w1_copy.start()
        w2_copy.start()

        def wqkv_transpose(p):
            a, b = QP[p]
            wqkvt_ref[a // 2:b // 2, :] = _pk(wqkv_ref[:, a:b].T)

        k_ref[0] = jnp.zeros((D, 128), f32)
        v_ref[0] = jnp.zeros((D, 128), f32)
        wof_ref[4] = jnp.zeros((D, 128), f32)

        x_copy(0).wait()
        layernorm(0, True)
        x_copy(1).wait()
        layernorm(1, True)

        wqkv_copy(0).wait()
        wqkv_transpose(0)
        qkv((0, 1), 0, 256)

        wqkv_copy(1).wait()
        qkv((0, 1), 256, 384)
        wqkv_transpose(1)
        qkv((0, 1), 384, 896)

        wqkv_copy(2).wait()
        for tt in range(2, 5):
            x_copy(tt).wait()
        qkv((0, 1), 896, 1024)
        wqkv_transpose(2)
        for tt in range(2, 5):
            layernorm(tt)
        qkv((0, 1), 1024, 1728)
        qkv((2, 3, 4), 0, 704)
        qkv((2, 3, 4), 704, 1408)

        for tt in range(5, 8):
            x_copy(tt).wait()
        wo_copy.wait()
        b1_copy.wait()
        w1_copy.wait()
        qkv((2, 3, 4), 1408, 1568)
        qkv((2, 3, 4), 1568, 1728)
        for tt in range(5, 8):
            layernorm(tt)

        w1t_ref[:, 0:512] = _pk(w1_ref[0:512, :].T)
        row = lax.broadcasted_iota(jnp.int32, (64, 128), 0)
        for c in range(F // 128):
            brow = jnp.where(row < 2, b1_ref[c:c + 1, :].astype(f32), 0.0).astype(bf16)
            blk = jnp.concatenate([w1_ref[512:576, c * 128:(c + 1) * 128], brow], axis=0)
            w1t_ref[c * 64:(c + 1) * 64, 512:640] = _pk(blk.T)
        for n in range(5):
            nw = min(128, D - n * 128)
            wof_ref[n, :, 0:nw] = wo_ref[:, n * 128:n * 128 + nw].astype(f32)
        for n in range(5):
            nw = min(128, D - n * 128)
            blk = jnp.concatenate(
                [wof_ref[n, pl.ds(d, H, stride=DH), :] for d in range(DH)], axis=0)
            wopt_ref[n * 64:n * 64 + nw // 2, :] = _pk(blk.T[0:nw, :].astype(bf16))

        qkv((5, 6, 7), 0, 864)
        qkv((5, 6, 7), 864, 1728)
        w2_copy.wait()

    @pl.when(step > 0)
    def _phase_b():
        i = step - 1
        cexp = (DH ** -0.5) / LOG2E
        neg = -1e9 * (DH ** 0.5) * LOG2E * LOG2E
        lane = lax.broadcasted_iota(jnp.int32, (G, 128), 1)

        def shifted(prev, cur, w):
            if w == 0:
                return cur
            return pltpu.roll(jnp.where(lane >= 128 - DIL * w, prev, cur), DIL * w, 1)

        for j in range(NB):
            jb = i * NB + j
            for g in range(H // G):
                logits = [None] * W
                for d in range(DH):
                    rows = pl.ds(d + g * G * DH, G, stride=DH)
                    q = q_ref[jb, rows, :]
                    prev = k_ref[jb, rows, :]
                    cur = k_ref[jb + 1, rows, :]
                    for w in range(W):
                        t = q * shifted(prev, cur, w)
                        logits[w] = t if logits[w] is None else logits[w] + t
                if j == 0:
                    pos = i * T + lane
                    for w in range(1, W):
                        logits[w] = jnp.where(pos >= DIL * w, logits[w], neg)
                m = logits[0]
                for w in range(1, W):
                    m = jnp.maximum(m, logits[w])
                p = [jnp.exp2((l - m) * cexp) for l in logits]
                den = p[0]
                for w in range(1, W):
                    den = den + p[w]
                inv = 1.0 / den
                p = [pw * inv for pw in p]
                for d in range(DH):
                    rows = pl.ds(d + g * G * DH, G, stride=DH)
                    prev = v_ref[jb, rows, :]
                    cur = v_ref[jb + 1, rows, :]
                    o = None
                    for w in range(W):
                        t = p[w] * shifted(prev, cur, w)
                        o = t if o is None else o + t
                    o_ref[d * H + g * G:d * H + (g + 1) * G, j * 128:(j + 1) * 128] = o.astype(bf16)

        xg = _unpk(xg_ref[i])
        acc = None
        lo = 0
        for n in F_CHUNKS:
            hi = lo + n
            g = jnp.dot(_unpk(w1t_ref[lo // 2:hi // 2, :]), xg, preferred_element_type=f32)
            a = _mish2(g).astype(bf16)
            y = jnp.dot(w2t_ref[:, lo:hi], a, preferred_element_type=f32)
            acc = y if acc is None else acc + y
            lo = hi
        acc = acc + jnp.dot(_unpk(wopt_ref[...]), o_ref[...], preferred_element_type=f32)
        out_ref[...] = (acc * (1.0 / LOG2E) + x_ref[i].astype(f32)).astype(bf16)


@jax.jit
def pallas_parallel_sum__sliding_local_dilated__dense_activation_mish__prompt_kernel(
    A_x: jax.Array,
    A_wqkv: jax.Array,
    A_wo: jax.Array,
    B_x: jax.Array,
    B_w1: jax.Array,
    B_b1: jax.Array,
    B_w2: jax.Array,
):
    del B_x
    xt = jnp.swapaxes(A_x, 1, 2)
    w2t = B_w2.T
    b1 = B_b1.reshape(F // 128, 128)
    out_t = pl.pallas_call(
        _kernel,
        grid=(NT + 1,),
        in_specs=[pl.BlockSpec(memory_space=pl.ANY)] * 6,
        out_specs=pl.BlockSpec((None, D, T), lambda s: (0, 0, jnp.maximum(s - 1, 0))),
        out_shape=jax.ShapeDtypeStruct((1, D, S), bf16),
        scratch_shapes=[
            pltpu.VMEM((NT, D, T), bf16),
            pltpu.VMEM((D, 3 * D), bf16),
            pltpu.VMEM((D, D), bf16),
            pltpu.VMEM((D, F), bf16),
            pltpu.VMEM((F // 128, 128), bf16),
            pltpu.VMEM((D, F), bf16),
            pltpu.VMEM((F // 2, KP), u32),
            pltpu.VMEM((3 * D // 2, D), u32),
            pltpu.VMEM((5, D, 128), f32),
            pltpu.VMEM((D // 2, D), u32),
            pltpu.VMEM((NT, KP // 2, T), u32),
            pltpu.VMEM((S // 128, D, 128), f32),
            pltpu.VMEM((S // 128 + 1, D, 128), f32),
            pltpu.VMEM((S // 128 + 1, D, 128), f32),
            pltpu.VMEM((D, T), bf16),
            pltpu.SemaphoreType.DMA((NT + 7,)),
        ],
        compiler_params=pltpu.CompilerParams(
            dimension_semantics=("arbitrary",),
            vmem_limit_bytes=64 * 1024 * 1024,
        ),
    )(xt, A_wqkv, A_wo, B_w1, b1, w2t)
    return jnp.swapaxes(out_t, 1, 2)
```

```python
import jax
import jax.numpy as jnp
from jax import lax
import jax.experimental.pallas as pl
import jax.experimental.pallas.tpu as pltpu

S, D, F = 2048, 576, 4608
H, DH, W, DIL = 32, 18, 8, 2
T = 256
NT = S // T
NB = T // 128
KP = 640
G = 8
F_CHUNKS = (2560, 1024, 1024)
QP = ((0, 384), (384, 1024), (1024, 1728))
EPS = 1e-5
LOG2E = 1.4426950408889634
LOG2E_HI = 1.4453125
LOG2E_LO = LOG2E - LOG2E_HI

f32 = jnp.float32
bf16 = jnp.bfloat16
u32 = jnp.uint32


def _pk(x):
    return pltpu.bitcast(x, u32)


def _unpk(x):
    return pltpu.bitcast(x, bf16)


def _mish2(g):
    e = jnp.exp2(jnp.minimum(g, 40.0))
    n = e * (e + 2.0)
    return g * (n * pl.reciprocal(n + 2.0, approx=True))


def _kernel(x_hbm, wqkv_hbm, wo_hbm, w1_hbm, b1_hbm, w2t_hbm, out_ref,
            x_ref, wqkv_ref, wo_ref, w1_ref, b1_ref, w2t_ref,
            w1t_ref, wqkvt_ref, wof_ref, wopt_ref, xg_ref, q_ref, k_ref, v_ref, o_ref, sems):
    step = pl.program_id(0)

    def x_copy(tt):
        return pltpu.make_async_copy(x_hbm.at[0, :, pl.ds(tt * T, T)], x_ref.at[tt], sems.at[tt])

    def wqkv_copy(p):
        a, b = QP[p]
        return pltpu.make_async_copy(
            wqkv_hbm.at[:, pl.ds(a, b - a)], wqkv_ref.at[:, pl.ds(a, b - a)], sems.at[NT + p])

    def layernorm(tt, fast=False):
        if fast:
            def colsum(parts):
                while len(parts) > 1:
                    parts = [parts[k] + parts[k + 1] for k in range(0, len(parts) - 1, 2)] + (
                        [parts[-1]] if len(parts) % 2 else [])
                return jnp.sum(parts[0], axis=0, keepdims=True)

            n1, n2, n3 = D // 4, D // 6, D // 3
            mean = colsum([jnp.sum(x_ref[tt, a:a + n1, :].astype(f32).reshape(n1 // 8, 8, T), axis=0)
                           for a in range(0, D, n1)]) * (1.0 / D)
            parts = []
            for a in range(0, D, n2):
                xc = x_ref[tt, a:a + n2, :].astype(f32) - mean
                parts.append(jnp.sum((xc * xc).reshape(n2 // 8, 8, T), axis=0))
            rstd = lax.rsqrt(colsum(parts) * (1.0 / D) + EPS) * LOG2E
            for a in range(0, D, n3):
                xc = x_ref[tt, a:a + n3, :].astype(f32) - mean
                xg_ref[tt, a // 2:(a + n3) // 2, :] = _pk((xc * rstd).astype(bf16))
        else:
            x = x_ref[tt].astype(f32)
            mean = jnp.sum(x, axis=0, keepdims=True) * (1.0 / D)
            xc = x - mean
            rstd = lax.rsqrt(jnp.sum(xc * xc, axis=0, keepdims=True) * (1.0 / D) + EPS) * LOG2E
            xg_ref[tt, 0:D // 2, :] = _pk((xc * rstd).astype(bf16))
        row = lax.broadcasted_iota(jnp.int32, (KP - D, T), 0)
        xg_ref[tt, D // 2:KP // 2, :] = _pk(
            jnp.where(row == 0, LOG2E_HI, jnp.where(row == 1, LOG2E_LO, 0.0)).astype(bf16))

    def qkv(tiles, a, b, wt=None):
        xg = _unpk(jnp.concatenate([xg_ref[tt, 0:D // 2, :] for tt in tiles], axis=1))
        if wt is None:
            wt = _unpk(wqkvt_ref[a // 2:b // 2, :])
        val = jnp.dot(wt, xg, preferred_element_type=f32)
        for sec, ref, off in ((0, q_ref, 0), (1, k_ref, 1), (2, v_ref, 1)):
            lo, hi = max(a, sec * D), min(b, (sec + 1) * D)
            if lo >= hi:
                continue
            for j in range(len(tiles) * NB):
                ref[tiles[0] * NB + j + off, lo - sec * D:hi - sec * D, :] = (
                    val[lo - a:hi - a, j * 128:(j + 1) * 128])

    @pl.when(step == 0)
    def _phase_a():
        wo_copy = pltpu.make_async_copy(wo_hbm, wo_ref, sems.at[NT + 3])
        b1_copy = pltpu.make_async_copy(b1_hbm, b1_ref, sems.at[NT + 4])
        w1_copy = pltpu.make_async_copy(w1_hbm, w1_ref, sems.at[NT + 5])
        w2_copy = pltpu.make_async_copy(w2t_hbm, w2t_ref, sems.at[NT + 6])

        x_copy(0).start()
        x_copy(1).start()
        for p in range(3):
            wqkv_copy(p).start()
        for tt in range(2, NT):
            x_copy(tt).start()
        wo_copy.start()
        b1_copy.start()
        w1_copy.start()
        w2_copy.start()

        def wqkv_transpose(p):
            a, b = QP[p]
            wqkvt_ref[a // 2:b // 2, :] = _pk(wqkv_ref[:, a:b].T)

        k_ref[0] = jnp.zeros((D, 128), f32)
        wof_ref[4] = jnp.zeros((D, 128), f32)

        x_copy(0).wait()
        layernorm(0, True)
        x_copy(1).wait()
        layernorm(1, True)

        wqkv_copy(0).wait()
        wt0 = wqkv_ref[:, 0:128].T
        qkv((0, 1), 0, 128, wt0)
        wqkvt_ref[0:64, :] = _pk(wt0)
        wqkvt_ref[64:192, :] = _pk(wqkv_ref[:, 128:384].T)
        qkv((0, 1), 128, 320)

        wqkv_copy(1).wait()
        qkv((0, 1), 320, 384)
        wqkv_transpose(1)
        qkv((0, 1), 384, 960)

        wqkv_copy(2).wait()
        for tt in range(2, 5):
            x_copy(tt).wait()
        qkv((0, 1), 960, 1024)
        wqkv_transpose(2)
        for tt in range(2, 5):
            layernorm(tt)
        qkv((0, 1), 1024, 1728)
        qkv((2, 3, 4), 0, 704)
        qkv((2, 3, 4), 704, 1408)

        for tt in range(5, 8):
            x_copy(tt).wait()
        wo_copy.wait()
        b1_copy.wait()
        w1_copy.wait()
        v_ref[0] = jnp.broadcast_to(v_ref[1, :, 0:1], (D, 128))
        qkv((2, 3, 4), 1408, 1568)
        qkv((2, 3, 4), 1568, 1728)
        for tt in range(5, 8):
            layernorm(tt)

        w1t_ref[:, 0:512] = _pk(w1_ref[0:512, :].T)
        row = lax.broadcasted_iota(jnp.int32, (64, 128), 0)
        for c in range(F // 128):
            brow = jnp.where(row < 2, b1_ref[c:c + 1, :].astype(f32), 0.0).astype(bf16)
            blk = jnp.concatenate([w1_ref[512:576, c * 128:(c + 1) * 128], brow], axis=0)
            w1t_ref[c * 64:(c + 1) * 64, 512:640] = _pk(blk.T)
        for n in range(5):
            nw = min(128, D - n * 128)
            wof_ref[n, :, 0:nw] = wo_ref[:, n * 128:n * 128 + nw].astype(f32)
        for n in range(5):
            nw = min(128, D - n * 128)
            blk = jnp.concatenate(
                [wof_ref[n, pl.ds(d, H, stride=DH), :] for d in range(DH)], axis=0)
            wopt_ref[n * 64:n * 64 + nw // 2, :] = _pk(blk.T[0:nw, :].astype(bf16))

        qkv((5, 6, 7), 0, 864)
        qkv((5, 6, 7), 864, 1728)
        w2_copy.wait()

    @pl.when(step > 0)
    def _phase_b():
        i = step - 1
        cexp = (DH ** -0.5) / LOG2E
        neg = -1e9 * (DH ** 0.5) * LOG2E * LOG2E
        lane = lax.broadcasted_iota(jnp.int32, (G, 128), 1)

        def shifted(prev, cur, w):
            if w == 0:
                return cur
            return pltpu.roll(jnp.where(lane >= 128 - DIL * w, prev, cur), DIL * w, 1)

        for j in range(NB):
            jb = i * NB + j
            for g in range(H // G):
                logits = [None] * W
                for d in range(DH):
                    rows = pl.ds(d + g * G * DH, G, stride=DH)
                    q = q_ref[jb, rows, :]
                    prev = k_ref[jb, rows, :]
                    cur = k_ref[jb + 1, rows, :]
                    for w in range(W):
                        t = q * shifted(prev, cur, w)
                        logits[w] = t if logits[w] is None else logits[w] + t
                if j == 0:
                    pos = i * T + lane
                    for w in range(1, W):
                        logits[w] = jnp.where(pos >= DIL * w, logits[w], neg)
                m = logits[0]
                for w in range(1, W):
                    m = jnp.maximum(m, logits[w])
                p = [jnp.exp2((l - m) * cexp) for l in logits]
                den = p[0]
                for w in range(1, W):
                    den = den + p[w]
                inv = 1.0 / den
                p = [pw * inv for pw in p]
                for d in range(DH):
                    rows = pl.ds(d + g * G * DH, G, stride=DH)
                    prev = v_ref[jb, rows, :]
                    cur = v_ref[jb + 1, rows, :]
                    o = None
                    for w in range(W):
                        t = p[w] * shifted(prev, cur, w)
                        o = t if o is None else o + t
                    o_ref[d * H + g * G:d * H + (g + 1) * G, j * 128:(j + 1) * 128] = o.astype(bf16)

        xg = _unpk(xg_ref[i])
        acc = None
        lo = 0
        for n in F_CHUNKS:
            hi = lo + n
            g = jnp.dot(_unpk(w1t_ref[lo // 2:hi // 2, :]), xg, preferred_element_type=f32)
            a = _mish2(g).astype(bf16)
            y = jnp.dot(w2t_ref[:, lo:hi], a, preferred_element_type=f32)
            acc = y if acc is None else acc + y
            lo = hi
        acc = acc + jnp.dot(_unpk(wopt_ref[...]), o_ref[...], preferred_element_type=f32)
        out_ref[...] = (acc * (1.0 / LOG2E) + x_ref[i].astype(f32)).astype(bf16)


@jax.jit
def pallas_parallel_sum__sliding_local_dilated__dense_activation_mish__prompt_kernel(
    A_x: jax.Array,
    A_wqkv: jax.Array,
    A_wo: jax.Array,
    B_x: jax.Array,
    B_w1: jax.Array,
    B_b1: jax.Array,
    B_w2: jax.Array,
):
    del B_x
    xt = jnp.swapaxes(A_x, 1, 2)
    w2t = B_w2.T
    b1 = B_b1.reshape(F // 128, 128)
    out_t = pl.pallas_call(
        _kernel,
        grid=(NT + 1,),
        in_specs=[pl.BlockSpec(memory_space=pl.ANY)] * 6,
        out_specs=pl.BlockSpec((None, D, T), lambda s: (0, 0, jnp.maximum(s - 1, 0))),
        out_shape=jax.ShapeDtypeStruct((1, D, S), bf16),
        scratch_shapes=[
            pltpu.VMEM((NT, D, T), bf16),
            pltpu.VMEM((D, 3 * D), bf16),
            pltpu.VMEM((D, D), bf16),
            pltpu.VMEM((D, F), bf16),
            pltpu.VMEM((F // 128, 128), bf16),
            pltpu.VMEM((D, F), bf16),
            pltpu.VMEM((F // 2, KP), u32),
            pltpu.VMEM((3 * D // 2, D), u32),
            pltpu.VMEM((5, D, 128), f32),
            pltpu.VMEM((D // 2, D), u32),
            pltpu.VMEM((NT, KP // 2, T), u32),
            pltpu.VMEM((S // 128, D, 128), f32),
            pltpu.VMEM((S // 128 + 1, D, 128), f32),
            pltpu.VMEM((S // 128 + 1, D, 128), f32),
            pltpu.VMEM((D, T), bf16),
            pltpu.SemaphoreType.DMA((NT + 7,)),
        ],
        compiler_params=pltpu.CompilerParams(
            dimension_semantics=("arbitrary",),
            vmem_limit_bytes=64 * 1024 * 1024,
            disable_bounds_checks=True,
            disable_semaphore_checks=True,
        ),
    )(xt, A_wqkv, A_wo, B_w1, b1, w2t)
    return jnp.swapaxes(out_t, 1, 2)
```
